```python
import jax
import jax.numpy as jnp

def _softmax(x, axis=-1):
    return jax.nn.softmax(x, axis=axis)
def _gelu(x):
    return jax.nn.gelu(x, approximate=True)
def _silu(x):
    return jax.nn.silu(x)
def _sigmoid(x):
    return jax.nn.sigmoid(x)
def _layernorm(x, axis=-1, eps=1e-5):
    m = jnp.mean(x, axis=axis, keepdims=True)
    v = jnp.var(x, axis=axis, keepdims=True)
    return (x - m) / jnp.sqrt(v + eps)
def _scatter_add(tgt, idx, src, axis=0):
    return tgt.at[idx].add(src)
def _segment_sum(src, seg, n):
    return jax.ops.segment_sum(src, seg, n)
class _Rng:
    def __init__(self, key):
        self._k = key
    def _next(self):
        self._k, sub = jax.random.split(self._k)
        return sub
    def normal(self, shape):
        return jax.random.normal(self._next(), shape, dtype=jnp.bfloat16)
    def randint(self, lo, hi, shape):
        return jax.random.randint(self._next(), shape, lo, hi, dtype=jnp.int32)
    def uniform(self, shape, lo=0.0, hi=1.0):
        return jax.random.uniform(self._next(), shape, jnp.bfloat16, lo, hi)
    def permutation(self, n):
        return jax.random.permutation(self._next(), n)


kernel_name = 'recurrent_scan__ssm_conv_h3__mixer_token_mlp__prompt'

def setup_inputs():
    _rng = _Rng(jax.random.key(int.from_bytes(__import__("os").urandom(4), "little")))
    _w = (lambda a: (lambda t: t.astype(jnp.bfloat16) if jnp.issubdtype(t.dtype, jnp.floating) else t)(jnp.asarray(a)))
    def _A_setup():
        B, S, D = 1, 2048, 576
        ks = 4
        return {
            "q": _w((lambda *s: _rng.normal(s) * 0.05)(B, S, D)),
            "k": _w((lambda *s: _rng.normal(s) * 0.05)(B, S, D)),
            "v": _w((lambda *s: _rng.normal(s) * 0.05)(B, S, D)),
            "shift_k": _w((lambda *s: _rng.normal(s) * 0.05)(D, ks) * 0.5),
            "ssm_k": _w((lambda *s: _rng.normal(s) * 0.05)(D, S) * (1.0 / S ** 0.5)),
            "ssm_D": _w((lambda *s: _rng.normal(s) * 0.05)(D)),
        }
    _A_in = _A_setup()

    def _B_setup():
        B, S, D, F = 1, 2048, 576, 4608
        return {
            "x": _w((lambda *s: _rng.normal(s) * 0.05)(B, S, D)),
            "w1": _w((lambda *s: _rng.normal(s) * 0.05)(S, F) * (S ** -0.5)),
            "b1": _w((lambda *s: _rng.normal(s) * 0.05)(F) * 0.02),
            "w2": _w((lambda *s: _rng.normal(s) * 0.05)(F, S) * (F ** -0.5)),
            "b2": _w((lambda *s: _rng.normal(s) * 0.05)(S) * 0.02),
        }
    _B_in = _B_setup()

    return {
        "A_q": _A_in["q"],
        "A_k": _A_in["k"],
        "A_v": _A_in["v"],
        "A_shift_k": _A_in["shift_k"],
        "A_ssm_k": _A_in["ssm_k"],
        "A_ssm_D": _A_in["ssm_D"],
        "B_x": _B_in["x"],
        "B_w1": _B_in["w1"],
        "B_b1": _B_in["b1"],
        "B_w2": _B_in["w2"],
        "B_b2": _B_in["b2"],
    }

def reference(A_q, A_k, A_v, A_shift_k, A_ssm_k, A_ssm_D, B_x, B_w1, B_b1, B_w2, B_b2):
    def _A_ref(q, k, v, shift_k, ssm_k, ssm_D):
        B, S, D = q.shape
        ks = shift_k.shape[-1]
        k_pad = jnp.pad(k, ((0, 0), (ks - 1, 0), (0, 0)))
        k_shift = jnp.zeros_like(k)
        for t in range(ks):
            k_shift = k_shift + k_pad[:, t:t + S, :] * shift_k[:, ks - 1 - t][None, None, :]
        kv = k_shift * v
        L = 2 * S
        kv_pad = jnp.pad(kv, ((0, 0), (0, S), (0, 0)))
        kf_pad = jnp.pad(ssm_k, ((0, 0), (0, S)))
        kv_f = (lambda x, axes=(-2,-1): jnp.fft.rfft2(x.astype(jnp.float32), axes=axes))(kv_pad[:, None, :, :], axes=(1, 2))
        kf_f = (lambda x, axes=(-2,-1): jnp.fft.rfft2(x.astype(jnp.float32), axes=axes))(kf_pad[:, None, :], axes=(1, 2))
        kf_f = (lambda x, *d: x.transpose(*d))(kf_f, 1, 2, 0)
        y_f = kv_f * kf_f[None, :, :, :]
        y = (lambda x, s, axes=(-2,-1): jnp.fft.irfft2(x, s=s, axes=axes).astype(jnp.bfloat16))(y_f, (1, L), axes=(1, 2))[:, 0, :S, :]
        y = y + kv * ssm_D[None, None, :]
        return q * y

    def _B_ref(x, w1, b1, w2, b2):
        B, S, D = x.shape
        h = _layernorm(x, axis=-1)
        u = jnp.einsum("bsd,sf->bdf", h, w1) + b1
        u = _gelu(u)
        y = jnp.einsum("bdf,fs->bds", u, w2) + b2
        return (lambda x, *d: x.transpose(*d))(y, 0, 2, 1)

    x = A_q
    xn = _layernorm(x, axis=-1)
    s = _A_ref(xn, A_k, A_v, A_shift_k, A_ssm_k, A_ssm_D)
    g = _silu(_B_ref(xn, B_w1, B_b1, B_w2, B_b2))
    return x + s * g
```

```python
import functools

import jax
import jax.numpy as jnp
import numpy as np
import jax.experimental.pallas as pl
import jax.experimental.pallas.tpu as pltpu

C = 128
EPS = 1e-5


def _dft_tables():
    n = np.arange(C)[:, None]
    f = np.arange(C)[None, :]
    ang = np.pi * (((2 * f + 1) * n) % (4 * C)) / (2 * C)
    fw = np.concatenate([np.cos(ang), -np.sin(ang)], axis=1)
    inv = fw.T / C
    return fw.astype(jnp.bfloat16), np.ascontiguousarray(inv).astype(jnp.bfloat16)


def _ln_rows(x):
    d = x.shape[0]
    m = jnp.sum(x, axis=0, keepdims=True) * (1.0 / d)
    xc = x - m
    v = jnp.sum(xc * xc, axis=0, keepdims=True) * (1.0 / d)
    return xc * jax.lax.rsqrt(v + EPS)


def _gelu(x):
    c0 = float(np.sqrt(2.0 / np.pi))
    return 0.5 * x * (1.0 + jnp.tanh(c0 * (x + 0.044715 * (x * x * x))))


def _silu(x):
    return x * jax.nn.sigmoid(x)


def _col(row, n):
    return jnp.broadcast_to(row, (C, n)).T


def _kernel(x_ref, k_ref, v_ref, sk_ref, ssm_ref, d_ref, w1_ref, b1_ref, w2_ref, b2_ref,
            fw_ref, inv_ref, o_ref,
            ht_ref, xn_ref, y_ref, acc_ref, tap_ref,
            *, S, D, G, nsteps):
    step = pl.program_id(0)
    M = S // C
    f32 = jnp.float32
    bf16 = jnp.bfloat16
    ks = sk_ref.shape[0]

    @pl.when(step == 0)
    def _prologue():
        for c in range(M):
            sl = slice(c * C, (c + 1) * C)
            xn = _ln_rows(x_ref[:, sl].astype(f32)).astype(bf16)
            xn_ref[:, sl] = xn
            ht_ref[:, sl] = _ln_rows(xn.astype(f32)).astype(bf16)
        sk = sk_ref[...].astype(f32)
        for j in range(ks):
            tap_ref[j] = _col(sk[j:j + 1, :], D)
        tap_ref[ks] = _col(d_ref[...].astype(f32), D)

    g0 = pl.multiple_of(step * G, G)
    rows = pl.ds(g0, G)
    kf = k_ref[...].astype(f32)
    pos = jax.lax.broadcasted_iota(jnp.int32, (1, S), 1)
    taps = [tap_ref[j, rows, :] for j in range(ks)]
    rolled = [kf] + [jnp.where(pos >= j, pltpu.roll(kf, j, axis=1), 0.0) for j in range(1, ks)]
    vf = v_ref[...].astype(f32)
    kv = []
    for c in range(M):
        sl = slice(c * C, (c + 1) * C)
        t = rolled[0][:, sl] * taps[0]
        for j in range(1, ks):
            t = t + rolled[j][:, sl] * taps[j]
        kv.append((t * vf[:, sl]).astype(bf16))
    xs = jnp.concatenate(kv, axis=0)
    fw = fw_ref[...]
    kst = jnp.concatenate([ssm_ref[:, m * C:(m + 1) * C] for m in range(M)], axis=0)
    kf_all = jnp.dot(kst, fw, preferred_element_type=f32)
    xf_all = jnp.dot(xs, fw, preferred_element_type=f32)
    lane = jax.lax.broadcasted_iota(jnp.int32, (1, C), 1)
    sgn = (1 - 2 * (lane & 1)).astype(f32)
    kr = [kf_all[m * G:(m + 1) * G, :C] for m in range(M)]
    ki = [kf_all[m * G:(m + 1) * G, C:] for m in range(M)]
    kr[0] = kr[0] + tap_ref[ks, rows, :]
    xr0 = [xf_all[m * G:(m + 1) * G, :C] for m in range(M)]
    xi0 = [xf_all[m * G:(m + 1) * G, C:] for m in range(M)]
    xr = [xr0[0]] + [xr0[a] - sgn * xi0[a - 1] for a in range(1, M)]
    xi = [xi0[0]] + [xi0[a] + sgn * xr0[a - 1] for a in range(1, M)]
    ys = []
    for i in range(M):
        yr = kr[0] * xr[i] - ki[0] * xi[i]
        yi = kr[0] * xi[i] + ki[0] * xr[i]
        for m in range(1, i + 1):
            yr = yr + (kr[m] * xr[i - m] - ki[m] * xi[i - m])
            yi = yi + (kr[m] * xi[i - m] + ki[m] * xr[i - m])
        ys.append(jnp.concatenate([yr, yi], axis=1).astype(bf16))
    ycat = jnp.concatenate(ys, axis=0)
    y = jnp.dot(ycat, inv_ref[...], preferred_element_type=f32)
    for c in range(M):
        y_ref[rows, c * C:(c + 1) * C] = y[c * G:(c + 1) * G, :].astype(bf16)

    u = jnp.dot(ht_ref[...], w1_ref[...], preferred_element_type=f32) + b1_ref[...].astype(f32)
    u = _gelu(u).astype(bf16)
    part = jnp.dot(u, w2_ref[...], preferred_element_type=f32)

    @pl.when(step == 0)
    def _():
        acc_ref[...] = part + b2_ref[...].astype(f32)

    @pl.when(step > 0)
    def _():
        acc_ref[...] += part

    @pl.when(step == nsteps - 1)
    def _epilogue():
        for c in range(M):
            sl = slice(c * C, (c + 1) * C)
            g = _silu(acc_ref[:, sl])
            s = xn_ref[:, sl].astype(f32) * y_ref[:, sl].astype(f32)
            o_ref[:, sl] = (x_ref[:, sl].astype(f32) + s * g).astype(o_ref.dtype)


@jax.jit
def pallas_recurrent_scan__ssm_conv_h3__mixer_token_mlp__prompt_kernel(
    A_q: jax.Array,
    A_k: jax.Array,
    A_v: jax.Array,
    A_shift_k: jax.Array,
    A_ssm_k: jax.Array,
    A_ssm_D: jax.Array,
    B_x: jax.Array,
    B_w1: jax.Array,
    B_b1: jax.Array,
    B_w2: jax.Array,
    B_b2: jax.Array,
):
    del B_x
    B, S, D = A_q.shape
    assert B == 1
    F = B_w1.shape[1]
    nsteps = 9
    TF = F // nsteps
    G = D // nsteps
    ks = A_shift_k.shape[1]
    fw, inv = _dft_tables()
    full = lambda shape: pl.BlockSpec(shape, lambda i: (0,) * len(shape))
    tr = lambda a: a.reshape(S, D).T
    out = pl.pallas_call(
        functools.partial(_kernel, S=S, D=D, G=G, nsteps=nsteps),
        grid=(nsteps,),
        in_specs=[
            full((D, S)),
            pl.BlockSpec((G, S), lambda i: (i, 0)),
            pl.BlockSpec((G, S), lambda i: (i, 0)),
            full((ks, D)),
            pl.BlockSpec((G, S), lambda i: (i, 0)),
            full((1, D)),
            pl.BlockSpec((S, TF), lambda i: (0, i)),
            pl.BlockSpec((1, TF), lambda i: (0, i)),
            pl.BlockSpec((TF, S), lambda i: (i, 0)),
            full((1, S)),
            full((C, 2 * C)), full((2 * C, C)),
        ],
        out_specs=full((D, S)),
        out_shape=jax.ShapeDtypeStruct((D, S), A_q.dtype),
        scratch_shapes=[
            pltpu.VMEM((D, S), jnp.bfloat16),
            pltpu.VMEM((D, S), jnp.bfloat16),
            pltpu.VMEM((D, S), jnp.bfloat16),
            pltpu.VMEM((D, S), jnp.float32),
            pltpu.VMEM((ks + 1, D, C), jnp.float32),
        ],
        compiler_params=pltpu.CompilerParams(
            dimension_semantics=("arbitrary",),
            vmem_limit_bytes=100 * 1024 * 1024,
        ),
    )(tr(A_q), tr(A_k), tr(A_v), A_shift_k.T, A_ssm_k,
      A_ssm_D.reshape(1, D), B_w1, B_b1.reshape(1, F), B_w2, B_b2.reshape(1, S), fw, inv)
    return out.T.reshape(B, S, D)
```

```python
import jax
import jax.numpy as jnp
import numpy as np
import jax.experimental.pallas as pl
import jax.experimental.pallas.tpu as pltpu

C = 128
EPS = 1e-5
NSTEPS = 12
NX = 8
NOUT = 16
MAC_ROWS = 16


def _dft_tables():
    n = np.arange(C)[:, None]
    f = np.arange(C)[None, :]
    ang = np.pi * (((2 * f + 1) * n) % (4 * C)) / (2 * C)
    fw = np.concatenate([np.cos(ang), -np.sin(ang)], axis=1)
    inv = fw.T / C
    return fw.astype(jnp.bfloat16), np.ascontiguousarray(inv).astype(jnp.bfloat16)


def _ln_rows(x):
    d = x.shape[0]
    m = jnp.sum(x, axis=0, keepdims=True) * (1.0 / d)
    xc = x - m
    v = jnp.sum(xc * xc, axis=0, keepdims=True) * (1.0 / d)
    return xc * jax.lax.rsqrt(v + EPS)


def _gelu(x):
    c0 = float(np.sqrt(2.0 / np.pi))
    return 0.5 * x * (1.0 + jnp.tanh(c0 * (x + 0.044715 * (x * x * x))))


def _silu(x):
    return 0.5 * x * (1.0 + jnp.tanh(0.5 * x))


def _col(row):
    return jnp.broadcast_to(row, (C, row.shape[1])).T


def _aligned(i, n):
    return i * n if isinstance(i, int) else pl.multiple_of(i * n, n)


def _start(cps, priority=0):
    for c in cps:
        c.start(priority=priority)


def _wait(cps):
    for c in cps:
        c.wait()


def _kernel(x_hbm, k_hbm, v_hbm, sk_hbm, ssm_hbm, d_hbm, w1_hbm, b1_hbm, w2_hbm, b2_hbm,
            fw_hbm, inv_hbm, zero_ref, o_hbm,
            xbuf, w1buf, w2buf, kbuf, vbuf, sbuf, skbuf, dbuf, b1buf, b2buf, fw_ref, inv_ref,
            ht_ref, xn_ref, y_ref, acc_ref, uacc_ref, ubuf, tap_ref, b1f_ref, xf_ref,
            sem, xsem, osem, ssem):
    f32, bf16 = jnp.float32, jnp.bfloat16
    D, S = xbuf.shape
    F = w1_hbm.shape[1]
    ks = sk_hbm.shape[0]
    TF, G, M = F // NSTEPS, D // NSTEPS, S // C
    NT, XW, OW = TF // C, S // NX, S // NOUT
    lane = jax.lax.broadcasted_iota(jnp.int32, (1, C), 1)

    def cp_w1(j):
        return [pltpu.make_async_copy(w1_hbm.at[:, pl.ds(_aligned(j, TF), TF)], w1buf.at[j % 2],
                                      sem.at[j % 2])]

    def cp_w2(j):
        return [pltpu.make_async_copy(w2_hbm.at[pl.ds(_aligned(j, TF), TF), :], w2buf.at[j % 2],
                                      sem.at[2 + j % 2])]

    def cp_kvs(j):
        r, s = pl.ds(_aligned(j, G), G), j % 2
        return [pltpu.make_async_copy(k_hbm.at[r, :], kbuf.at[s], sem.at[4 + s]),
                pltpu.make_async_copy(v_hbm.at[r, :], vbuf.at[s], sem.at[6 + s]),
                pltpu.make_async_copy(ssm_hbm.at[r, :], sbuf.at[s], sem.at[8 + s])]

    def cp_x(p):
        cols = pl.ds(_aligned(p, XW), XW)
        return pltpu.make_async_copy(x_hbm.at[:, cols], xbuf.at[:, cols], xsem.at[p])

    def cp_w1_rows(p):
        rows = pl.ds(_aligned(p, XW), XW)
        return pltpu.make_async_copy(w1_hbm.at[rows, pl.ds(0, TF)], w1buf.at[0, rows, :],
                                     xsem.at[NX + p])

    small = [pltpu.make_async_copy(src, dst, ssem.at[i]) for i, (src, dst) in enumerate((
        (sk_hbm, skbuf), (d_hbm, dbuf), (b1_hbm, b1buf), (b2_hbm, b2buf),
        (fw_hbm, fw_ref), (inv_hbm, inv_ref)))]

    def front(slot, rows):
        taps = [tap_ref[t, rows, :] for t in range(ks)]
        prev, out = None, []
        for c in range(M):
            sl = slice(c * C, (c + 1) * C)
            cur = kbuf[slot, :, sl].astype(f32)
            rot = [pltpu.roll(cur, t, axis=1) for t in range(1, ks)]
            acc = cur * taps[0]
            for t in range(1, ks):
                sh = jnp.where(lane >= t, rot[t - 1], 0.0 if prev is None else prev[t - 1])
                acc = acc + sh * taps[t]
            prev = rot
            out.append((acc * vbuf[slot, :, sl].astype(f32)).astype(bf16))
        return jnp.concatenate(out, axis=0)

    def fwd_k(slot, rows):
        kst = jnp.concatenate([sbuf[slot, :, m * C:(m + 1) * C] for m in range(M)], axis=0)
        kf = jnp.dot(kst, fw_ref[...], preferred_element_type=f32)
        kr = [kf[m * G:(m + 1) * G, :C] for m in range(M)]
        ki = [kf[m * G:(m + 1) * G, C:] for m in range(M)]
        kr[0] = kr[0] + tap_ref[ks, rows, :]
        return kr, ki

    def spectra_x(xs):
        xf = jnp.dot(xs, fw_ref[...], preferred_element_type=f32)
        sgn = (1 - 2 * (lane & 1)).astype(f32)
        re = [xf[a * G:(a + 1) * G, :C] for a in range(M)]
        im = [xf[a * G:(a + 1) * G, C:] for a in range(M)]
        xr = [re[0]] + [re[a] - sgn * im[a - 1] for a in range(1, M)]
        xi = [im[0]] + [im[a] + sgn * re[a - 1] for a in range(1, M)]
        return xr, xi

    def mac_values(kk, xx):
        (kr, ki), (xr, xi) = kk, xx
        ys = []
        for i in range(M):
            yr = kr[0] * xr[i] - ki[0] * xi[i]
            yi = kr[0] * xi[i] + ki[0] * xr[i]
            for m in range(1, i + 1):
                yr = yr + (kr[m] * xr[i - m] - ki[m] * xi[i - m])
                yi = yi + (kr[m] * xi[i - m] + ki[m] * xr[i - m])
            ys.append(jnp.concatenate([yr, yi], axis=1).astype(bf16))
        return jnp.concatenate(ys, axis=0)

    def park_x(xx):
        for a in range(M):
            xf_ref[0, a] = xx[0][a]
            xf_ref[1, a] = xx[1][a]

    def mac_in_place(kk):
        kr, ki = kk
        zero = zero_ref[0]
        for g in range(G // MAC_ROWS):
            rs = slice(g * MAC_ROWS, (g + 1) * MAC_ROWS)
            for i in range(M - 1, -1, -1):
                yr = yi = None
                for m in range(i + 1):
                    xr, xi = xf_ref[0, i - m, rs, :], xf_ref[1, i - m, rs, :]
                    pr = kr[m][rs] * xr - ki[m][rs] * xi
                    pi = kr[m][rs] * xi + ki[m][rs] * xr
                    yr, yi = (pr, pi) if m == 0 else (yr + pr, yi + pi)
                xf_ref[0, i + zero, rs, :] = yr
                xf_ref[1, i + zero, rs, :] = yi

    def parked_y():
        return jnp.concatenate(
            [jnp.concatenate([xf_ref[0, i], xf_ref[1, i]], axis=1).astype(bf16) for i in range(M)],
            axis=0)

    def inverse(ycat, rows):
        y = jnp.dot(ycat, inv_ref[...], preferred_element_type=f32)
        for c in range(M):
            y_ref[rows, c * C:(c + 1) * C] = y[c * G:(c + 1) * G, :].astype(bf16)

    def bias1(j):
        return jnp.concatenate([b1f_ref[pl.ds(j * NT + n, 1), :] for n in range(NT)], axis=1)

    def mm1(j):
        u = jnp.dot(ht_ref[...], w1buf[j % 2], preferred_element_type=f32) + bias1(j)
        return _gelu(u).astype(bf16)

    def layer_norms(p):
        for c in range(XW // C):
            sl = pl.ds(_aligned(p * (XW // C) + c, C), C)
            xn = _ln_rows(xbuf[:, sl].astype(f32)).astype(bf16)
            xn_ref[:, sl] = xn
            ht_ref[:, sl] = _ln_rows(xn.astype(f32)).astype(bf16)

    def mm1_first(p):
        sl = pl.ds(_aligned(p, XW), XW)
        return uacc_ref[...] + jnp.dot(ht_ref[:, sl], w1buf[0, sl, :], preferred_element_type=f32)

    for p in range(NX):
        cp_x(p).start()
        cp_w1_rows(p).start()
    _start(small + cp_kvs(0), priority=1)
    acc_ref[...] = jnp.zeros(acc_ref.shape, f32)
    uacc_ref[...] = jnp.zeros(uacc_ref.shape, f32)
    cp_x(0).wait()
    _start(cp_w2(0) + cp_kvs(1) + cp_w1(1), priority=1)
    layer_norms(0)

    def head_body(p, carry):
        cp_w1_rows(p).wait()
        cp_x(p + 1).wait()
        uacc_ref[...] = mm1_first(p)
        layer_norms(p + 1)
        return carry

    jax.lax.fori_loop(0, NX - 1, head_body, 0)
    cp_w1_rows(NX - 1).wait()
    _wait(small + cp_kvs(0))
    skf = skbuf[...].astype(f32)
    for t in range(ks):
        tap_ref[t] = _col(skf[t:t + 1, :])
    tap_ref[ks] = _col(dbuf[...].astype(f32).reshape(1, D))
    b1f_ref[...] = b1buf[...].astype(f32)
    ubuf[0] = _gelu(mm1_first(NX - 1) + bias1(0)).astype(bf16)
    rows0 = pl.ds(0, G)
    kk = fwd_k(0, rows0)
    inverse(mac_values(kk, spectra_x(front(0, rows0))), rows0)

    def body(j, carry):
        _start(cp_w2(j + 1))

        @pl.when(j + 2 < NSTEPS)
        def _():
            _start(cp_w1(j + 2) + cp_kvs(j + 2))

        _wait(cp_w2(j) + cp_w1(j + 1) + cp_kvs(j + 1))
        slot1 = (j + 1) % 2
        rows = pl.ds(_aligned(j + 1, G), G)
        kk = fwd_k(slot1, rows)
        xs = front(slot1, rows)
        park_x(spectra_x(xs))
        acc_ref[...] += jnp.dot(ubuf[j % 2], w2buf[j % 2], preferred_element_type=f32)
        mac_in_place(kk)
        ubuf[slot1] = mm1(j + 1)
        inverse(parked_y(), rows)
        return carry

    jax.lax.fori_loop(0, NSTEPS - 1, body, 0)

    last = NSTEPS - 1
    _wait(cp_w2(last))
    out_cps = []
    u = ubuf[last % 2]
    b2f = b2buf[...].astype(f32)
    for p in range(NOUT):
        cols = slice(p * OW, (p + 1) * OW)
        b2 = jnp.concatenate([b2f[n:n + 1, :] for n in range(p * OW // C, (p + 1) * OW // C)], axis=1)
        part = jnp.dot(u, w2buf[last % 2, :, cols], preferred_element_type=f32)
        g = _silu(acc_ref[:, cols] + part + b2)
        s = xn_ref[:, cols].astype(f32) * y_ref[:, cols].astype(f32)
        xbuf[:, cols] = (xbuf[:, cols].astype(f32) + s * g).astype(bf16)
        cp = pltpu.make_async_copy(xbuf.at[:, cols], o_hbm.at[:, cols], osem.at[p])
        cp.start()
        out_cps.append(cp)
    _wait(out_cps)


@jax.jit
def pallas_recurrent_scan__ssm_conv_h3__mixer_token_mlp__prompt_kernel(
    A_q: jax.Array,
    A_k: jax.Array,
    A_v: jax.Array,
    A_shift_k: jax.Array,
    A_ssm_k: jax.Array,
    A_ssm_D: jax.Array,
    B_x: jax.Array,
    B_w1: jax.Array,
    B_b1: jax.Array,
    B_w2: jax.Array,
    B_b2: jax.Array,
):
    del B_x
    B, S, D = A_q.shape
    F = B_w1.shape[1]
    ks = A_shift_k.shape[1]
    assert B == 1 and F % (NSTEPS * C) == 0 and D % (NSTEPS * 16) == 0 and S % (NOUT * C) == 0
    TF, G, M = F // NSTEPS, D // NSTEPS, S // C
    fw, inv = _dft_tables()
    bf16, f32 = jnp.bfloat16, jnp.float32
    hbm = pl.BlockSpec(memory_space=pl.ANY)

    def channel_major(a):
        return a.reshape(S, D).T

    out = pl.pallas_call(
        _kernel,
        in_specs=[hbm] * 12 + [pl.BlockSpec(memory_space=pltpu.SMEM)],
        out_specs=hbm,
        out_shape=jax.ShapeDtypeStruct((D, S), A_q.dtype),
        scratch_shapes=[
            pltpu.VMEM((D, S), bf16),
            pltpu.VMEM((2, S, TF), bf16),
            pltpu.VMEM((2, TF, S), bf16),
            pltpu.VMEM((2, G, S), bf16),
            pltpu.VMEM((2, G, S), bf16),
            pltpu.VMEM((2, G, S), bf16),
            pltpu.VMEM((ks, D), bf16),
            pltpu.VMEM((D,), bf16),
            pltpu.VMEM((F // C, C), bf16),
            pltpu.VMEM((S // C, C), bf16),
            pltpu.VMEM((C, 2 * C), bf16),
            pltpu.VMEM((2 * C, C), bf16),
            pltpu.VMEM((D, S), bf16),
            pltpu.VMEM((D, S), bf16),
            pltpu.VMEM((D, S), bf16),
            pltpu.VMEM((D, S), f32),
            pltpu.VMEM((D, TF), f32),
            pltpu.VMEM((2, D, TF), bf16),
            pltpu.VMEM((ks + 1, D, C), f32),
            pltpu.VMEM((F // C, C), f32),
            pltpu.VMEM((2, M, G, C), f32),
            pltpu.SemaphoreType.DMA((10,)),
            pltpu.SemaphoreType.DMA((2 * NX,)),
            pltpu.SemaphoreType.DMA((NOUT,)),
            pltpu.SemaphoreType.DMA((6,)),
        ],
        compiler_params=pltpu.CompilerParams(
            vmem_limit_bytes=100 * 1024 * 1024, disable_bounds_checks=True),
    )(channel_major(A_q), channel_major(A_k), channel_major(A_v), A_shift_k.T, A_ssm_k, A_ssm_D,
      B_w1, B_b1.reshape(F // C, C), B_w2, B_b2.reshape(S // C, C), fw, inv,
      np.zeros((1,), np.int32))
    return out.T.reshape(B, S, D)
```
